```python
import jax
import jax.numpy as jnp

def _softmax(x, axis=-1):
    return jax.nn.softmax(x, axis=axis)
def _gelu(x):
    return jax.nn.gelu(x, approximate=True)
def _silu(x):
    return jax.nn.silu(x)
def _sigmoid(x):
    return jax.nn.sigmoid(x)
def _layernorm(x, axis=-1, eps=1e-5):
    m = jnp.mean(x, axis=axis, keepdims=True)
    v = jnp.var(x, axis=axis, keepdims=True)
    return (x - m) / jnp.sqrt(v + eps)
def _scatter_add(tgt, idx, src, axis=0):
    return tgt.at[idx].add(src)
def _segment_sum(src, seg, n):
    return jax.ops.segment_sum(src, seg, n)
class _Rng:
    def __init__(self, key):
        self._k = key
    def _next(self):
        self._k, sub = jax.random.split(self._k)
        return sub
    def normal(self, shape):
        return jax.random.normal(self._next(), shape, dtype=jnp.bfloat16)
    def randint(self, lo, hi, shape):
        return jax.random.randint(self._next(), shape, lo, hi, dtype=jnp.int32)
    def uniform(self, shape, lo=0.0, hi=1.0):
        return jax.random.uniform(self._next(), shape, jnp.bfloat16, lo, hi)
    def permutation(self, n):
        return jax.random.permutation(self._next(), n)


kernel_name = 'standalone__layernorm_linear__prompt'

def setup_inputs():
    _rng = _Rng(jax.random.key(int.from_bytes(__import__("os").urandom(4), "little")))
    _w = (lambda a: (lambda t: t.astype(jnp.bfloat16) if jnp.issubdtype(t.dtype, jnp.floating) else t)(jnp.asarray(a)))
    B, S, D = 2, 2048, 1024
    return {
        "x": _w((lambda *s: _rng.normal(s) * 0.05)(B, S, D)),
        "g": _w((lambda *s: _rng.normal(s) * 0.05)(D) + 1.0),
        "b": _w((lambda *s: _rng.normal(s) * 0.05)(D)),
        "w": _w((lambda *s: _rng.normal(s) * 0.05)(D, D)),
    }

def reference(x, g, b, w):
    return (_layernorm(x, axis=-1) * g + b) @ w
```

```python
import jax
import jax.numpy as jnp
from jax import lax
import jax.experimental.pallas as pl
import jax.experimental.pallas.tpu as pltpu

_BM = 512
_SUB = 256
_EPS = 1e-5


def _kernel(x_ref, g_ref, b_ref, w_ref, o_ref):
    g = g_ref[...].astype(jnp.float32)
    b = b_ref[...].astype(jnp.float32)
    for i in range(_BM // _SUB):
        rows = slice(i * _SUB, (i + 1) * _SUB)
        x = x_ref[rows, :].astype(jnp.float32)
        m = jnp.mean(x, axis=-1, keepdims=True)
        xc = x - m
        v = jnp.mean(xc * xc, axis=-1, keepdims=True)
        y = xc * lax.rsqrt(v + _EPS) * g + b
        o_ref[rows, :] = jnp.dot(
            y.astype(w_ref.dtype), w_ref[...], preferred_element_type=jnp.float32
        ).astype(o_ref.dtype)


@jax.jit
def pallas_standalone__layernorm_linear__prompt_kernel(
    x: jax.Array,
    g: jax.Array,
    b: jax.Array,
    w: jax.Array,
):
    B, S, D = x.shape
    M = B * S
    N = w.shape[1]
    out = pl.pallas_call(
        _kernel,
        grid=(M // _BM,),
        in_specs=[
            pl.BlockSpec((_BM, D), lambda i: (i, 0)),
            pl.BlockSpec((1, D), lambda i: (0, 0)),
            pl.BlockSpec((1, D), lambda i: (0, 0)),
            pl.BlockSpec((D, N), lambda i: (0, 0)),
        ],
        out_specs=pl.BlockSpec((_BM, N), lambda i: (i, 0)),
        out_shape=jax.ShapeDtypeStruct((M, N), x.dtype),
        compiler_params=pltpu.CompilerParams(
            dimension_semantics=("arbitrary",),
            vmem_limit_bytes=64 * 1024 * 1024,
        ),
    )(x.reshape(M, D), g.reshape(1, D), b.reshape(1, D), w)
    return out.reshape(B, S, N)
```

```python
import jax
import jax.numpy as jnp
from jax import lax
import jax.experimental.pallas as pl
import jax.experimental.pallas.tpu as pltpu

_EPS = 1e-5
_LANES = 128
_R = 16
_C = 128
_P0 = 256
_KPH = 4
_LEAD = 2
_NP1 = 3
_NIT = 3
_LAG = 2
_CHAINS = 2
_SPLIT = 4

f32 = jnp.float32
bf16 = jnp.bfloat16
u32 = jnp.uint32


def _ln_piece(xb, g, b, zero):
    d = xb.shape[1]
    x = xb.astype(f32)
    tiles = [x[:, c:c + _LANES] for c in range(0, d, _LANES)]
    s = tiles[0] if zero is None else tiles[0] + pltpu.bitcast(zero, f32)
    for t in tiles[1:]:
        s = s + t
    mean = jnp.sum(s, axis=-1, keepdims=True) * (1.0 / d)
    xc = [t - mean for t in tiles]
    q = xc[0] * xc[0]
    for t in xc[1:]:
        q = q + t * t
    var = jnp.sum(q, axis=-1, keepdims=True) * (1.0 / d)
    rstd = lax.rsqrt(var + _EPS)
    ys = [
        xc[i] * rstd * g[:, i * _LANES:(i + 1) * _LANES] + b[:, i * _LANES:(i + 1) * _LANES]
        for i in range(len(tiles))
    ]
    return jnp.concatenate(ys, axis=-1), ys[-1]


def _make_kernel(M, D, N):
    c, R, L = _C, _R, _LEAD
    NT = N // _LANES
    q0 = _P0 // c
    per_it = (M // c - q0 - _NP1) // _NIT
    assert q0 + _NP1 + per_it * _NIT == M // c
    NB = L + 1
    assert per_it % NB == 0 and c // R == NT and L <= _KPH
    ks = D // _KPH
    groups = [(0, _P0)] + [((q0 + l) * c, c) for l in range(L)] + [((q0 + L) * c, _NP1 * c)]
    for it in range(_NIT):
        lo = (q0 + _NP1 + L + it * per_it) * c
        groups.append((lo, min(lo + per_it * c, M) - lo))
    g_p1 = 1 + L
    g_it = g_p1 + 1

    def kernel(x_hbm, g_hbm, b_hbm, w_hbm, o_hbm,
               x_v, o_v, w_v, xn, xn0, acc, g_v, b_v, z_v,
               sem_x, sem_o, sem_w, sem_gb, sem_f):

        def x_copy(j):
            rows = pl.ds(*groups[j])
            return pltpu.make_async_copy(x_hbm.at[rows], x_v.at[rows], sem_x.at[j])

        def w_copy(k):
            rows = pl.ds(k * ks, ks)
            return pltpu.make_async_copy(w_hbm.at[rows], w_v.at[rows], sem_w.at[k])

        def o_copy(r0, nr, c0=0, nc=N):
            if nc == N:
                idx = (pl.ds(r0, nr),)
            else:
                idx = (pl.ds(r0, nr), pl.ds(c0, nc))
            return pltpu.make_async_copy(o_v.at[idx], o_hbm.at[idx], sem_o.at[0])

        g_copy = pltpu.make_async_copy(g_hbm, g_v, sem_gb.at[0])
        b_copy = pltpu.make_async_copy(b_hbm, b_v, sem_gb.at[1])

        seq = [g_copy, b_copy, x_copy(0)]
        for k in range(_KPH):
            if k - (_KPH - L) >= 0:
                seq.append(x_copy(1 + k - (_KPH - L)))
            seq.append(w_copy(k))
        seq += [x_copy(j) for j in range(g_p1, len(groups))]
        for cp in seq:
            cp.start()
            pl.semaphore_signal(sem_f, 1)
            pl.semaphore_wait(sem_f, 1)
        z_v[...] = jnp.zeros_like(z_v)
        g_copy.wait()
        b_copy.wait()
        x_copy(0).wait()

        def load_gb():
            return (g_v[...].astype(f32).reshape(1, D), b_v[...].astype(f32).reshape(1, D))

        g, b = load_gb()
        for r in range(0, _P0, R):
            xn0[r:r + R, :] = _ln_piece(x_v[r:r + R, :], g, b, None)[0].astype(bf16)

        st = {}

        def new_region():
            st["zero"] = z_v[...]
            st["mm"] = []
            st["ln"] = []
            st["g"], st["b"] = load_gb()

        def chunk_step(ln_base, dst, mm_fn, after_piece=None):
            for n in range(NT):
                if ln_base is not None:
                    z = st["zero"]
                    if len(st["mm"]) >= _LAG:
                        z = st["mm"][-_LAG]
                    if len(st["ln"]) >= _CHAINS:
                        z = z & st["ln"][-_CHAINS]
                    y, ylast = _ln_piece(x_v[pl.ds(ln_base + n * R, R), :], st["g"], st["b"], z)
                    dst[n * R:(n + 1) * R, :] = y.astype(bf16)
                    st["ln"].append(st["zero"] & pltpu.bitcast(ylast, u32))
                res = mm_fn(n)
                if ln_base is not None:
                    st["mm"].append(st["zero"] & pltpu.bitcast(res[0:R, :], u32))
                if after_piece is not None:
                    after_piece(n)

        for k in range(_KPH):
            l = k - (_KPH - L)
            w_copy(k).wait()
            if l >= 0:
                x_copy(1 + l).wait()

            def mm_slab(n, k=k):
                cols = slice(n * _LANES, (n + 1) * _LANES)
                res = jnp.dot(xn0[:, k * ks:(k + 1) * ks], w_v[k * ks:(k + 1) * ks, cols],
                              preferred_element_type=f32)
                if k > 0:
                    res = res + acc[:, cols]
                if k == _KPH - 1:
                    o_v[0:_P0, cols] = res.astype(bf16)
                else:
                    acc[:, cols] = res
                return res

            new_region()
            if l >= 0:
                chunk_step((q0 + l) * c, xn.at[(q0 + l) % NB], mm_slab)
            else:
                chunk_step(None, None, mm_slab)

        def run_chunks(qs, nchunks, row0, clamp, issue_out):
            for t in range(nchunks):
                q = qs + t
                rbase = row0 + t * c
                lnb = rbase + L * c
                if clamp and t >= nchunks - L:
                    lnb = jnp.minimum(lnb, M - c)
                if not isinstance(rbase, int):
                    rbase = pl.multiple_of(rbase, c)
                    lnb = pl.multiple_of(lnb, c)
                src = xn.at[q % NB]
                dst = xn.at[(q + L) % NB]

                def mm_tile(n, src=src, rbase=rbase):
                    cols = slice(n * _LANES, (n + 1) * _LANES)
                    res = jnp.dot(src[...], w_v[:, cols], preferred_element_type=f32)
                    o_v[pl.ds(rbase, c), cols] = res.astype(bf16)
                    return res

                parts = _SPLIT if t == nchunks - 1 else 1

                def after(n, rbase=rbase, parts=parts):
                    if issue_out and (n + 1) % (NT // parts) == 0:
                        j = n // (NT // parts)
                        o_copy(rbase, c, j * (N // parts), N // parts).start()

                chunk_step(lnb, dst, mm_tile, after)

        x_copy(g_p1).wait()
        new_region()
        run_chunks(q0, _NP1, _P0, False, False)

        def body(i, carry):
            for it in range(_NIT):
                @pl.when(i == it)
                def _():
                    x_copy(g_it + it).wait()
                    if it == 0:
                        o_copy(0, _P0 + _NP1 * c).start()
            new_region()
            row0 = (q0 + _NP1) * c + i * (per_it * c)
            run_chunks(q0 + _NP1, per_it, row0, True, True)
            return carry

        lax.fori_loop(0, _NIT, body, 0)
        pltpu.make_async_copy(o_v, o_hbm, sem_o.at[0]).wait()

    scratch = [
        pltpu.VMEM((M, D), bf16),
        pltpu.VMEM((M, N), bf16),
        pltpu.VMEM((D, N), bf16),
        pltpu.VMEM((NB, c, D), bf16),
        pltpu.VMEM((_P0, D), bf16),
        pltpu.VMEM((_P0, N), f32),
        pltpu.VMEM((D,), bf16),
        pltpu.VMEM((D,), bf16),
        pltpu.VMEM((R, _LANES), u32),
        pltpu.SemaphoreType.DMA((len(groups),)),
        pltpu.SemaphoreType.DMA((1,)),
        pltpu.SemaphoreType.DMA((_KPH,)),
        pltpu.SemaphoreType.DMA((2,)),
        pltpu.SemaphoreType.REGULAR,
    ]
    return kernel, scratch


@jax.jit
def pallas_standalone__layernorm_linear__prompt_kernel(
    x: jax.Array,
    g: jax.Array,
    b: jax.Array,
    w: jax.Array,
):
    B, S, D = x.shape
    M = B * S
    N = w.shape[1]
    kernel, scratch = _make_kernel(M, D, N)
    out = pl.pallas_call(
        kernel,
        in_specs=[pl.BlockSpec(memory_space=pl.ANY)] * 4,
        out_specs=pl.BlockSpec(memory_space=pl.ANY),
        out_shape=jax.ShapeDtypeStruct((M, N), x.dtype),
        scratch_shapes=scratch,
        compiler_params=pltpu.CompilerParams(vmem_limit_bytes=48 * 1024 * 1024),
    )(x.reshape(M, D), g, b, w)
    return out.reshape(B, S, N)
```

```python
import jax
import jax.numpy as jnp
from jax import lax
import jax.experimental.pallas as pl
import jax.experimental.pallas.tpu as pltpu

_EPS = 1e-5
_LANES = 128
_R = 16
_C = 128
_P0 = 256
_KSLABS = 4
_LEAD = 2
_NIT = 3
_LAG = 2
_CHAINS = 2
_SPLIT = 8
_LN_LAST_SLAB = 2
_PRE = (((2,), (3,)), ((3, 4), (4, 5, 6)))

f32 = jnp.float32
bf16 = jnp.bfloat16
u32 = jnp.uint32


def _ln_piece(xb, g, b, zero):
    d = xb.shape[1]
    x = xb.astype(f32)
    tiles = [x[:, c:c + _LANES] for c in range(0, d, _LANES)]
    s = tiles[0] if zero is None else tiles[0] + pltpu.bitcast(zero, f32)
    for t in tiles[1:]:
        s = s + t
    mean = jnp.sum(s, axis=-1, keepdims=True) * (1.0 / d)
    xc = [t - mean for t in tiles]
    q = xc[0] * xc[0]
    for t in xc[1:]:
        q = q + t * t
    var = jnp.sum(q, axis=-1, keepdims=True) * (1.0 / d)
    rstd = lax.rsqrt(var + _EPS)
    ys = [
        xc[i] * rstd * g[:, i * _LANES:(i + 1) * _LANES] + b[:, i * _LANES:(i + 1) * _LANES]
        for i in range(len(tiles))
    ]
    return jnp.concatenate(ys, axis=-1), ys[-1]


def _make_kernel(M, D, N):
    c, R, L = _C, _R, _LEAD
    NT = N // _LANES
    ks = D // _KSLABS
    first_loop = _P0 // c + sum(len(mm) for mm, _ in _PRE)
    per_it = (M // c - first_loop) // _NIT
    NB = L + 1
    assert first_loop + per_it * _NIT == M // c and per_it % NB == 0

    groups = [(0, _P0), (_LN_LAST_SLAB * c, c)]
    groups += [(ln[0] * c, len(ln) * c) for _, ln in _PRE]
    for it in range(_NIT):
        lo = (first_loop + L + it * per_it) * c
        groups.append((lo, min(lo + per_it * c, M) - lo))
    g_pre = 2
    g_it = g_pre + len(_PRE)

    def kernel(x_hbm, g_hbm, b_hbm, w_hbm, o_hbm,
               x_v, o_v, w_v, w32, xn32, xn0, acc, g_v, b_v, z_v,
               sem_x, sem_o, sem_w, sem_gb, sem_f):

        def x_copy(j):
            rows = pl.ds(*groups[j])
            return pltpu.make_async_copy(x_hbm.at[rows], x_v.at[rows], sem_x.at[j])

        def w_copy(k):
            rows = pl.ds(k * ks, ks)
            return pltpu.make_async_copy(w_hbm.at[rows], w_v.at[rows], sem_w.at[k])

        def o_copy(r0, nr, c0=0, nc=N):
            idx = (pl.ds(r0, nr),) if nc == N else (pl.ds(r0, nr), pl.ds(c0, nc))
            return pltpu.make_async_copy(o_v.at[idx], o_hbm.at[idx], sem_o.at[0])

        g_copy = pltpu.make_async_copy(g_hbm, g_v, sem_gb.at[0])
        b_copy = pltpu.make_async_copy(b_hbm, b_v, sem_gb.at[1])

        seq = [g_copy, b_copy, x_copy(0)]
        seq += [w_copy(k) for k in range(_KSLABS - 1)]
        seq += [x_copy(1), w_copy(_KSLABS - 1)]
        seq += [x_copy(j) for j in range(g_pre, len(groups))]
        for cp in seq:
            cp.start()
            pl.semaphore_signal(sem_f, 1)
            pl.semaphore_wait(sem_f, 1)
        z_v[...] = jnp.zeros_like(z_v)
        g_copy.wait()
        b_copy.wait()
        x_copy(0).wait()

        def load_gb():
            return (g_v[...].astype(f32).reshape(1, D), b_v[...].astype(f32).reshape(1, D))

        g, b = load_gb()
        for r in range(0, _P0, R):
            xn0[r:r + R, :] = _ln_piece(x_v[r:r + R, :], g, b, None)[0].astype(bf16)

        def region(mm_pieces, ln_chunks, after=None):
            zero = z_v[...]
            g, b = load_gb()
            mm_done, ln_done = [], []
            todo = [(base, dst, j) for base, dst in ln_chunks for j in range(c // R)]
            pos = [(i * len(mm_pieces)) // len(todo) for i in range(len(todo))]
            i = 0
            for n, mm in enumerate(mm_pieces):
                while i < len(todo) and pos[i] == n:
                    base, dst, j = todo[i]
                    z = mm_done[-_LAG] if len(mm_done) >= _LAG else zero
                    if len(ln_done) >= _CHAINS:
                        z = z & ln_done[-_CHAINS]
                    y, ylast = _ln_piece(x_v[pl.ds(base + j * R, R), :], g, b, z)
                    dst[j * R // 2:(j + 1) * R // 2, :] = pltpu.bitcast(y.astype(bf16), u32)
                    ln_done.append(zero & pltpu.bitcast(ylast, u32))
                    i += 1
                res = mm()
                mm_done.append(zero & pltpu.bitcast(res[0:R, :], u32))
                if after is not None:
                    after(n, mm_done[-1])

        for k in range(_KSLABS):
            last = k == _KSLABS - 1
            w_copy(k).wait()
            if last:
                x_copy(1).wait()
            kk = slice(k * ks, (k + 1) * ks)

            def slab_piece(n, k=k, kk=kk, last=last):
                def f():
                    cols = slice(n * _LANES, (n + 1) * _LANES)
                    res = jnp.dot(xn0[:, kk], w_v[kk, cols], preferred_element_type=f32)
                    if k > 0:
                        res = res + acc[:, cols]
                    if last:
                        o_v[0:_P0, cols] = res.astype(bf16)
                    else:
                        acc[:, cols] = res
                    return res
                return f

            def repack(n, zero, k=k):
                zrow = jnp.concatenate([zero[0:8, :]] * NT, axis=1)
                for r in range(k * ks + n * (ks // NT), k * ks + (n + 1) * (ks // NT), 16):
                    w32[r // 2:r // 2 + 8, :] = pltpu.bitcast(w_v[r:r + 16, :], u32) | zrow

            ln = [(_LN_LAST_SLAB * c, xn32.at[_LN_LAST_SLAB % NB])] if last else []
            region([slab_piece(n) for n in range(NT)], ln, repack)

        def chunk_pieces(q, row):
            def piece(n):
                def f():
                    cols = slice(n * _LANES, (n + 1) * _LANES)
                    lhs = pltpu.bitcast(xn32.at[q % NB][...], bf16)
                    rhs = pltpu.bitcast(w32[:, cols], bf16)
                    res = jnp.dot(lhs, rhs, preferred_element_type=f32)
                    o_v[pl.ds(row, c), cols] = res.astype(bf16)
                    return res
                return f
            return [piece(n) for n in range(NT)]

        for j, (mm, ln) in enumerate(_PRE):
            x_copy(g_pre + j).wait()
            region([f for q in mm for f in chunk_pieces(q, q * c)],
                   [(q * c, xn32.at[q % NB]) for q in ln])

        def body(i, carry):
            for it in range(_NIT):
                @pl.when(i == it)
                def _():
                    x_copy(g_it + it).wait()
                    if it == 0:
                        o_copy(0, first_loop * c).start()
            row0 = first_loop * c + i * (per_it * c)
            pieces, ln = [], []
            for t in range(per_it):
                q = first_loop + t
                pieces += chunk_pieces(q, pl.multiple_of(row0 + t * c, c))
                ln_row = row0 + (t + L) * c
                if t >= per_it - L:
                    ln_row = jnp.minimum(ln_row, M - c)
                ln.append((pl.multiple_of(ln_row, c), xn32.at[(q + L) % NB]))

            def send(n, _):
                t, nn = divmod(n, NT)
                parts = _SPLIT if t == per_it - 1 else 1
                if (nn + 1) % (NT // parts) == 0:
                    j = nn // (NT // parts)
                    o_copy(pl.multiple_of(row0 + t * c, c), c, j * (N // parts), N // parts).start()

            region(pieces, ln, send)
            return carry

        lax.fori_loop(0, _NIT, body, 0)
        pltpu.make_async_copy(o_v, o_hbm, sem_o.at[0]).wait()

    scratch = [
        pltpu.VMEM((M, D), bf16),
        pltpu.VMEM((M, N), bf16),
        pltpu.VMEM((D, N), bf16),
        pltpu.VMEM((D // 2, N), u32),
        pltpu.VMEM((NB, c // 2, D), u32),
        pltpu.VMEM((_P0, D), bf16),
        pltpu.VMEM((_P0, N), f32),
        pltpu.VMEM((D,), bf16),
        pltpu.VMEM((D,), bf16),
        pltpu.VMEM((R, _LANES), u32),
        pltpu.SemaphoreType.DMA((len(groups),)),
        pltpu.SemaphoreType.DMA((1,)),
        pltpu.SemaphoreType.DMA((_KSLABS,)),
        pltpu.SemaphoreType.DMA((2,)),
        pltpu.SemaphoreType.REGULAR,
    ]
    return kernel, scratch


@jax.jit
def pallas_standalone__layernorm_linear__prompt_kernel(
    x: jax.Array,
    g: jax.Array,
    b: jax.Array,
    w: jax.Array,
):
    B, S, D = x.shape
    M = B * S
    N = w.shape[1]
    kernel, scratch = _make_kernel(M, D, N)
    out = pl.pallas_call(
        kernel,
        in_specs=[pl.BlockSpec(memory_space=pl.ANY)] * 4,
        out_specs=pl.BlockSpec(memory_space=pl.ANY),
        out_shape=jax.ShapeDtypeStruct((M, N), x.dtype),
        scratch_shapes=scratch,
        compiler_params=pltpu.CompilerParams(
            vmem_limit_bytes=48 * 1024 * 1024,
            disable_semaphore_checks=True,
        ),
    )(x.reshape(M, D), g, b, w)
    return out.reshape(B, S, N)
```

```python
import jax
import jax.numpy as jnp
from jax import lax
import jax.experimental.pallas as pl
import jax.experimental.pallas.tpu as pltpu

_EPS = 1e-5
_LANES = 128
_R = 16
_C = 128
_P0 = 256
_KSLABS = 4
_LEAD = 2
_NIT = 2
_LAG = 2
_CHAINS = 2
_SPLIT = 8
_LN_LAST_SLAB = 2
_FENCED_SLABS = (0, 1, 3)
_PRE = (((2,), (3,)), ((3, 4), (4, 5)), ((5, 6, 7), (6, 7, 8, 9)))

f32 = jnp.float32
bf16 = jnp.bfloat16
u32 = jnp.uint32


def _ln_piece(xb, g, b, zero):
    d = xb.shape[1]
    x = xb.astype(f32)
    tiles = [x[:, c:c + _LANES] for c in range(0, d, _LANES)]
    s = tiles[0] if zero is None else tiles[0] + pltpu.bitcast(zero, f32)
    for t in tiles[1:]:
        s = s + t
    mean = jnp.sum(s, axis=-1, keepdims=True) * (1.0 / d)
    xc = [t - mean for t in tiles]
    q = xc[0] * xc[0]
    for t in xc[1:]:
        q = q + t * t
    var = jnp.sum(q, axis=-1, keepdims=True) * (1.0 / d)
    rstd = lax.rsqrt(var + _EPS)
    ys = [
        xc[i] * rstd * g[:, i * _LANES:(i + 1) * _LANES] + b[:, i * _LANES:(i + 1) * _LANES]
        for i in range(len(tiles))
    ]
    return jnp.concatenate(ys, axis=-1), ys[-1]


def _make_kernel(M, D, N):
    c, R, L = _C, _R, _LEAD
    NT = N // _LANES
    ks = D // _KSLABS
    first_loop = _P0 // c + sum(len(mm) for mm, _ in _PRE)
    per_it = (M // c - first_loop) // _NIT
    NB = L + 1
    assert first_loop + per_it * _NIT == M // c and per_it % NB == 0

    groups = [(0, _P0), (_LN_LAST_SLAB * c, c)]
    groups += [(ln[0] * c, len(ln) * c) for _, ln in _PRE]
    for it in range(_NIT):
        lo = (first_loop + L + it * per_it) * c
        groups.append((lo, min(lo + per_it * c, M) - lo))
    g_pre = 2
    g_it = g_pre + len(_PRE)

    def kernel(x_hbm, g_hbm, b_hbm, w_hbm, o_hbm,
               x_v, o_v, w_v, w32, xn32, xn0, acc, g_v, b_v, z_v,
               sem_x, sem_o, sem_w, sem_gb, sem_f):

        def x_copy(j):
            rows = pl.ds(*groups[j])
            return pltpu.make_async_copy(x_hbm.at[rows], x_v.at[rows], sem_x.at[j])

        def w_copy(k):
            rows = pl.ds(k * ks, ks)
            return pltpu.make_async_copy(w_hbm.at[rows], w_v.at[rows], sem_w.at[k])

        def o_copy(r0, nr, c0=0, nc=N):
            idx = (pl.ds(r0, nr),) if nc == N else (pl.ds(r0, nr), pl.ds(c0, nc))
            return pltpu.make_async_copy(o_v.at[idx], o_hbm.at[idx], sem_o.at[0])

        g_copy = pltpu.make_async_copy(g_hbm, g_v, sem_gb.at[0])
        b_copy = pltpu.make_async_copy(b_hbm, b_v, sem_gb.at[1])

        seq = [g_copy, b_copy, x_copy(0)]
        seq += [w_copy(k) for k in range(_KSLABS - 1)]
        seq += [x_copy(1), w_copy(_KSLABS - 1)]
        seq += [x_copy(j) for j in range(g_pre, len(groups))]
        def fence():
            pl.semaphore_signal(sem_f, 1)
            pl.semaphore_wait(sem_f, 1)

        for cp in seq:
            cp.start()
            fence()
        z_v[...] = jnp.zeros_like(z_v)
        g_copy.wait()
        b_copy.wait()
        x_copy(0).wait()

        def load_gb():
            return (g_v[...].astype(f32).reshape(1, D), b_v[...].astype(f32).reshape(1, D))

        g, b = load_gb()
        for r in range(0, _P0, R):
            xn0[r:r + R, :] = _ln_piece(x_v[r:r + R, :], g, b, None)[0].astype(bf16)

        def region(mm_pieces, ln_chunks, after=None):
            zero = z_v[...]
            g, b = load_gb()
            mm_done, ln_done = [], []
            todo = [(base, dst, j) for base, dst in ln_chunks for j in range(c // R)]
            pos = [(i * len(mm_pieces)) // len(todo) for i in range(len(todo))]
            i = 0
            for n, mm in enumerate(mm_pieces):
                while i < len(todo) and pos[i] == n:
                    base, dst, j = todo[i]
                    z = mm_done[-_LAG] if len(mm_done) >= _LAG else zero
                    if len(ln_done) >= _CHAINS:
                        z = z & ln_done[-_CHAINS]
                    y, ylast = _ln_piece(x_v[pl.ds(base + j * R, R), :], g, b, z)
                    dst[j * R // 2:(j + 1) * R // 2, :] = pltpu.bitcast(y.astype(bf16), u32)
                    ln_done.append(zero & pltpu.bitcast(ylast, u32))
                    i += 1
                res = mm()
                mm_done.append(zero & pltpu.bitcast(res[0:R, :], u32))
                if after is not None:
                    after(n, mm_done[-1])

        for k in range(_KSLABS):
            last = k == _KSLABS - 1
            if k in _FENCED_SLABS:
                fence()
            w_copy(k).wait()
            if last:
                x_copy(1).wait()
            kk = slice(k * ks, (k + 1) * ks)

            def slab_piece(n, k=k, kk=kk, last=last):
                def f():
                    cols = slice(n * _LANES, (n + 1) * _LANES)
                    res = jnp.dot(xn0[:, kk], w_v[kk, cols], preferred_element_type=f32)
                    if k > 0:
                        res = res + acc[:, cols]
                    if last:
                        o_v[0:_P0, cols] = res.astype(bf16)
                    else:
                        acc[:, cols] = res
                    return res
                return f

            def repack(n, zero, k=k):
                zrow = jnp.concatenate([zero[0:8, :]] * NT, axis=1)
                for r in range(k * ks + n * (ks // NT), k * ks + (n + 1) * (ks // NT), 16):
                    w32[r // 2:r // 2 + 8, :] = pltpu.bitcast(w_v[r:r + 16, :], u32) | zrow

            ln = [(_LN_LAST_SLAB * c, xn32.at[_LN_LAST_SLAB % NB])] if last else []
            region([slab_piece(n) for n in range(NT)], ln, repack)

        def chunk_pieces(q, row):
            def piece(n):
                def f():
                    cols = slice(n * _LANES, (n + 1) * _LANES)
                    lhs = pltpu.bitcast(xn32.at[q % NB][...], bf16)
                    rhs = pltpu.bitcast(w32[:, cols], bf16)
                    res = jnp.dot(lhs, rhs, preferred_element_type=f32)
                    o_v[pl.ds(row, c), cols] = res.astype(bf16)
                    return res
                return f
            return [piece(n) for n in range(NT)]

        for j, (mm, ln) in enumerate(_PRE):
            x_copy(g_pre + j).wait()
            region([f for q in mm for f in chunk_pieces(q, q * c)],
                   [(q * c, xn32.at[q % NB]) for q in ln])

        def body(i, carry):
            for it in range(_NIT):
                @pl.when(i == it)
                def _():
                    x_copy(g_it + it).wait()
                    if it == 0:
                        o_copy(0, first_loop * c).start()
            row0 = first_loop * c + i * (per_it * c)
            pieces, ln = [], []
            for t in range(per_it):
                q = first_loop + t
                pieces += chunk_pieces(q, pl.multiple_of(row0 + t * c, c))
                ln_row = row0 + (t + L) * c
                if t >= per_it - L:
                    ln_row = jnp.minimum(ln_row, M - c)
                ln.append((pl.multiple_of(ln_row, c), xn32.at[(q + L) % NB]))

            def send(n, _):
                t, nn = divmod(n, NT)
                parts = _SPLIT if t == per_it - 1 else 1
                if (nn + 1) % (NT // parts) == 0:
                    j = nn // (NT // parts)
                    o_copy(pl.multiple_of(row0 + t * c, c), c, j * (N // parts), N // parts).start()

            region(pieces, ln, send)
            return carry

        lax.fori_loop(0, _NIT, body, 0)
        pltpu.make_async_copy(o_v, o_hbm, sem_o.at[0]).wait()

    scratch = [
        pltpu.VMEM((M, D), bf16),
        pltpu.VMEM((M, N), bf16),
        pltpu.VMEM((D, N), bf16),
        pltpu.VMEM((D // 2, N), u32),
        pltpu.VMEM((NB, c // 2, D), u32),
        pltpu.VMEM((_P0, D), bf16),
        pltpu.VMEM((_P0, N), f32),
        pltpu.VMEM((D,), bf16),
        pltpu.VMEM((D,), bf16),
        pltpu.VMEM((R, _LANES), u32),
        pltpu.SemaphoreType.DMA((len(groups),)),
        pltpu.SemaphoreType.DMA((1,)),
        pltpu.SemaphoreType.DMA((_KSLABS,)),
        pltpu.SemaphoreType.DMA((2,)),
        pltpu.SemaphoreType.REGULAR,
    ]
    return kernel, scratch


@jax.jit
def pallas_standalone__layernorm_linear__prompt_kernel(
    x: jax.Array,
    g: jax.Array,
    b: jax.Array,
    w: jax.Array,
):
    B, S, D = x.shape
    M = B * S
    N = w.shape[1]
    kernel, scratch = _make_kernel(M, D, N)
    out = pl.pallas_call(
        kernel,
        in_specs=[pl.BlockSpec(memory_space=pl.ANY)] * 4,
        out_specs=pl.BlockSpec(memory_space=pl.ANY),
        out_shape=jax.ShapeDtypeStruct((M, N), x.dtype),
        scratch_shapes=scratch,
        compiler_params=pltpu.CompilerParams(
            vmem_limit_bytes=48 * 1024 * 1024,
            disable_semaphore_checks=True,
            flags={"XLA_TPU_RESCHEDULE_DMA_DONES": True},
        ),
    )(x.reshape(M, D), g, b, w)
    return out.reshape(B, S, N)
```
